```python
import os as _os
_os.environ.setdefault("JAX_PLATFORMS", "cpu")
import jax
import jax.numpy as jnp

def _softmax(x, axis=-1):
    return jax.nn.softmax(x, axis=axis)
def _gelu(x):
    return jax.nn.gelu(x, approximate=True)
def _silu(x):
    return jax.nn.silu(x)
def _sigmoid(x):
    return jax.nn.sigmoid(x)
def _layernorm(x, axis=-1, eps=1e-5):
    m = jnp.mean(x, axis=axis, keepdims=True)
    v = jnp.var(x, axis=axis, keepdims=True)
    return (x - m) / jnp.sqrt(v + eps)
def _scatter_add(tgt, idx, src, axis=0):
    return tgt.at[idx].add(src)
def _segment_sum(src, seg, n):
    return jax.ops.segment_sum(src, seg, n)
class _Rng:
    def __init__(self, key):
        self._k = key
    def _next(self):
        self._k, sub = jax.random.split(self._k)
        return sub
    def normal(self, shape):
        return jax.random.normal(self._next(), shape, dtype=jnp.bfloat16)
    def randint(self, lo, hi, shape):
        return jax.random.randint(self._next(), shape, lo, hi, dtype=jnp.int32)
    def uniform(self, shape, lo=0.0, hi=1.0):
        return jax.random.uniform(self._next(), shape, jnp.bfloat16, lo, hi)
    def permutation(self, n):
        return jax.random.permutation(self._next(), n)


kernel_name = 'standalone__gqa_block_cached__near_ridge'

def setup_inputs():
    _rng = _Rng(jax.random.key(int.from_bytes(__import__("os").urandom(4), "little")))
    _w = (lambda a: (lambda t: t.astype(jnp.bfloat16) if jnp.issubdtype(t.dtype, jnp.floating) else t)(jnp.asarray(a)))
    B, Sq, D = 32, 112, 448
    Hq, Hkv, Sk, Dh = 16, 8, 512, 256
    assert Hq % Hkv == 0, (Hq, Hkv)
    return {
        "x": _w((lambda *s: _rng.normal(s) * 0.8)(B, Sq, D)),
        "k_cache": _w((lambda *s: _rng.normal(s) * 0.8)(B, Hkv, Sk, Dh)),
        "v_cache": _w((lambda *s: _rng.normal(s) * 0.05)(B, Hkv, Sk, Dh)),
        "wq": _w((lambda *s: _rng.normal(s) * 0.8)(D, Hq * Dh) * (D ** -0.5)),
        "wo": _w((lambda *s: _rng.normal(s) * 0.05)(Hq * Dh, D) * ((Hq * Dh) ** -0.5)),
    }

def reference(x, k_cache, v_cache, wq, wo):
    B, Sq, D = x.shape
    Hq, Dh = 16, 256
    Hkv = k_cache.shape[1]
    rep = Hq // Hkv
    q = (lambda x, *d: x.transpose(*d))((x @ wq).reshape(B, Sq, Hq, Dh), 0, 2, 1, 3)
    k = jnp.repeat(k_cache, rep, axis=1)
    v = jnp.repeat(v_cache, rep, axis=1)
    scores = jnp.einsum("bhqd,bhkd->bhqk", q, k) * (Dh ** -0.5)
    p = _softmax(scores, axis=-1)
    o = jnp.einsum("bhqk,bhkd->bhqd", p, v)
    return (lambda x, *d: x.transpose(*d))(o, 0, 2, 1, 3).reshape(B, Sq, Hq * Dh) @ wo
```

```python
import functools
import jax
import jax.numpy as jnp
import jax.experimental.pallas as pl
import jax.experimental.pallas.tpu as pltpu

RB = 896
CB = 1024
NB2 = 2
NSLOT = 10
MT = 4
LOG2E = 1.4426950408889634

f32 = jnp.float32
bf16 = jnp.bfloat16
NT = (((1,), (1,)), ((), ()))


def _kernel(x_hbm, k_hbm, v_hbm, wq_hbm, wot_hbm, out_hbm,
            x_v, wq_v, wot_v, q_v, k_v, v_v, out_v,
            sem_x, sem_wq, sem_wo, sem_k, sem_v, sem_o,
            *, B, sq, hq, hkv, dh):
    M, D = x_hbm.shape
    N = hq * dh
    rep = hq // hkv
    scale = (dh ** -0.5) * LOG2E
    nr, nc = M // RB, N // CB
    n1 = nr * nc
    n2 = B // NB2
    n3 = M // (128 * MT)

    def x_copy(r):
        return pltpu.make_async_copy(x_hbm.at[pl.ds(r * RB, RB), :], x_v.at[pl.ds(r * RB, RB), :], sem_x.at[r])

    def wq_copy(c):
        return pltpu.make_async_copy(wq_hbm.at[:, pl.ds(c * CB, CB)], wq_v.at[c], sem_wq.at[c])

    def wo_copy():
        return pltpu.make_async_copy(wot_hbm, wot_v, sem_wo.at[0])

    def k_copy(b, slot):
        return pltpu.make_async_copy(k_hbm.at[b], k_v.at[slot], sem_k.at[slot])

    def v_copy(b, slot):
        return pltpu.make_async_copy(v_hbm.at[b], v_v.at[slot], sem_v.at[slot])

    def out_copy(j):
        rows = pl.ds(j * (128 * MT), 128 * MT)
        return pltpu.make_async_copy(out_v.at[rows, :], out_hbm.at[rows, :], sem_o.at[j])

    x_copy(0).start()
    wq_copy(0).start()
    for r in range(1, nr):
        x_copy(r).start()
    for c in range(1, nc):
        wq_copy(c).start()

    def p1(i, carry):
        c = i // nr
        r = i % nr

        @pl.when(i < NSLOT)
        def _():
            k_copy(i, i).start()
            v_copy(i, i).start()

        @pl.when(i == NSLOT)
        def _():
            wo_copy().start()

        @pl.when(c == 0)
        def _():
            x_copy(r).wait()

        @pl.when(r == 0)
        def _():
            wq_copy(c).wait()

        r0 = pl.multiple_of(r * RB, 16)
        xb = x_v[pl.ds(r0, RB), :]
        for t in range(CB // dh):
            y = jnp.dot(xb, wq_v[c, :, t * dh:(t + 1) * dh], preferred_element_type=f32)
            q_v[c, pl.ds(r0, RB), t * dh:(t + 1) * dh] = (y * scale).astype(bf16)
        return carry

    jax.lax.fori_loop(0, n1, p1, 0)

    hpc = CB // dh

    def p2(i, carry):
        b0 = i * NB2

        @pl.when(i >= 1)
        def _():
            for u in range(NB2):
                bn = b0 - NB2 + u + NSLOT

                @pl.when(bn < B)
                def _():
                    slot = bn % NSLOT
                    k_copy(bn, slot).start()
                    v_copy(bn, slot).start()

        slots = []
        for u in range(NB2):
            slot = (b0 + u) % NSLOT
            k_copy(b0 + u, slot).wait()
            v_copy(b0 + u, slot).wait()
            slots.append(slot)

        r0 = pl.multiple_of(b0 * sq, 16)
        qv = q_v.at[:, pl.ds(r0, NB2 * sq), :]
        items = [(u, g) for u in range(NB2) for g in range(hkv)]
        n = len(items)

        def qslice(u, h):
            return (h // hpc, slice(u * sq, (u + 1) * sq), slice((h % hpc) * dh, (h % hpc + 1) * dh))

        def qk(j):
            u, g = items[j]
            q2 = jnp.concatenate([qv[qslice(u, g * rep + r)] for r in range(rep)], axis=0)
            return jax.lax.dot_general(q2, k_v[slots[u], g], NT, preferred_element_type=f32)

        def softmax(s):
            m = jnp.max(s, axis=-1, keepdims=True)
            p = jnp.exp2(s - m)
            l = jnp.sum(p, axis=-1, keepdims=True)
            return p.astype(bf16), l

        def pv(j, p, l):
            u, g = items[j]
            o = jnp.dot(p, v_v[slots[u], g], preferred_element_type=f32)
            o = (o * pl.reciprocal(l, approx=True)).astype(bf16)
            for r in range(rep):
                qv[qslice(u, g * rep + r)] = o[r * sq:(r + 1) * sq]

        s = qk(0)
        for j in range(n):
            s_next = qk(j + 1) if j + 1 < n else None
            p, l = softmax(s)
            pv(j, p, l)
            s = s_next
        return carry

    jax.lax.fori_loop(0, n2, p2, 0)

    wo_copy().wait()

    def p3(j, carry):
        @pl.when(j >= 1)
        def _():
            out_copy(j - 1).start()

        for t in range(MT):
            r0 = pl.multiple_of((j * MT + t) * 128, 128)
            acc = None
            for c in range(nc):
                part = jax.lax.dot_general(wot_v[:, c * CB:(c + 1) * CB], q_v[c, pl.ds(r0, 128), :], NT,
                                           preferred_element_type=f32)
                acc = part if acc is None else acc + part
            out_v[pl.ds(r0, 128), :] = acc.T.astype(bf16)
        return carry

    jax.lax.fori_loop(0, n3, p3, 0)
    out_copy(n3 - 1).start()
    for j in range(n3):
        out_copy(j).wait()


@jax.jit
def pallas_standalone__gqa_block_cached__near_ridge_kernel(x, k_cache, v_cache, wq, wo):
    B, Sq, D = x.shape
    _, Hkv, Sk, Dh = k_cache.shape
    N = wq.shape[1]
    Hq = N // Dh
    M = B * Sq
    kern = functools.partial(_kernel, B=B, sq=Sq, hq=Hq, hkv=Hkv, dh=Dh)
    hbm = lambda a: pltpu.with_memory_space_constraint(a, pltpu.HBM)
    any_spec = pl.BlockSpec(memory_space=pl.ANY)
    out = pl.pallas_call(
        kern,
        in_specs=[any_spec] * 5,
        out_specs=any_spec,
        out_shape=jax.ShapeDtypeStruct((M, D), x.dtype),
        scratch_shapes=[
            pltpu.VMEM((M, D), bf16),
            pltpu.VMEM((N // CB, D, CB), bf16),
            pltpu.VMEM((D, N), bf16),
            pltpu.VMEM((N // CB, M, CB), bf16),
            pltpu.VMEM((NSLOT, Hkv, Sk, Dh), bf16),
            pltpu.VMEM((NSLOT, Hkv, Sk, Dh), bf16),
            pltpu.VMEM((M, D), bf16),
            pltpu.SemaphoreType.DMA((M // RB,)),
            pltpu.SemaphoreType.DMA((N // CB,)),
            pltpu.SemaphoreType.DMA((1,)),
            pltpu.SemaphoreType.DMA((NSLOT,)),
            pltpu.SemaphoreType.DMA((NSLOT,)),
            pltpu.SemaphoreType.DMA((M // (128 * MT),)),
        ],
        compiler_params=pltpu.CompilerParams(
            vmem_limit_bytes=110 * 1024 * 1024,
        ),
    )(hbm(x.reshape(M, D)), hbm(k_cache), hbm(v_cache), hbm(wq), hbm(wo.T))
    return out.reshape(B, Sq, D)
```

```python
import functools
import jax
import jax.numpy as jnp
import jax.experimental.pallas as pl
import jax.experimental.pallas.tpu as pltpu

RA = 448
NB2 = 4
NGRP = 3
MT = 7
PERTILE = 1
LOG2E = 1.4426950408889634

f32 = jnp.float32
bf16 = jnp.bfloat16
NT = (((1,), (1,)), ((), ()))


def _kernel(x_hbm, k_hbm, v_hbm, wq_hbm, wot_hbm, out_hbm,
            x_v, wq_v, wot_v, q_v, k_v, v_v, out_v,
            sem_x, sem_wq, sem_wo, sem_k, sem_v, sem_o,
            *, B, sq, hq, hkv, dh):
    M, D = x_hbm.shape
    N = hq * dh
    rep = hq // hkv
    CB = rep * dh
    scale = (dh ** -0.5) * LOG2E
    RBk = M - RA
    n2 = B // NB2
    ntile = M // 128
    n3 = ntile // MT

    def x_copy(part):
        rows = pl.ds(0, RA) if part == 0 else pl.ds(RA, RBk)
        return pltpu.make_async_copy(x_hbm.at[rows, :], x_v.at[rows, :], sem_x.at[part])

    def wq_copy(c):
        return pltpu.make_async_copy(wq_hbm.at[:, pl.ds(c * CB, CB)], wq_v.at[c], sem_wq.at[c])

    def wo_copy():
        return pltpu.make_async_copy(wot_hbm, wot_v, sem_wo.at[0])

    def k_copy(i, grp):
        return pltpu.make_async_copy(k_hbm.at[pl.ds(i * NB2, NB2)], k_v.at[grp], sem_k.at[grp])

    def v_copy(i, grp):
        return pltpu.make_async_copy(v_hbm.at[pl.ds(i * NB2, NB2)], v_v.at[grp], sem_v.at[grp])

    def out_copy(tile, ntiles, s):
        rows = pl.ds(pl.multiple_of(tile * 128, 128), ntiles * 128)
        return pltpu.make_async_copy(out_v.at[rows, :], out_hbm.at[rows, :], sem_o.at[s])

    def qproj(r0, nrows, c):
        xb = x_v[pl.ds(r0, nrows), :]
        for t in range(rep):
            y = jnp.dot(xb, wq_v[c, :, t * dh:(t + 1) * dh], preferred_element_type=f32)
            q_v[c, pl.ds(r0, nrows), t * dh:(t + 1) * dh] = (y * scale).astype(bf16)

    x_copy(0).start()
    wq_copy(0).start()
    x_copy(0).wait()
    for c in range(1, hkv):
        wq_copy(c).start()
    x_copy(1).start()

    def p1a(c, carry):
        wq_copy(c).wait()
        qproj(0, RA, c)
        return carry

    jax.lax.fori_loop(0, hkv, p1a, 0)

    for grp in range(NGRP):
        k_copy(grp, grp).start()
        v_copy(grp, grp).start()
        if grp == min(1, NGRP - 1):
            wo_copy().start()
    x_copy(1).wait()

    def p1b(c, carry):
        qproj(RA, RBk, c)
        return carry

    jax.lax.fori_loop(0, hkv, p1b, 0)

    def p2(i, carry):
        grp = i % NGRP
        k_copy(i, grp).wait()
        v_copy(i, grp).wait()
        kg = k_v.at[grp]
        vg = v_v.at[grp]
        r0 = pl.multiple_of(i * (NB2 * sq), 16)
        qv = q_v.at[:, pl.ds(r0, NB2 * sq), :]
        items = [(u, g) for u in range(NB2) for g in range(hkv)]
        n = len(items)

        def qslice(u, g, r):
            return (g, slice(u * sq, (u + 1) * sq), slice(r * dh, (r + 1) * dh))

        def qk(j):
            u, g = items[j]
            q2 = jnp.concatenate([qv[qslice(u, g, r)] for r in range(rep)], axis=0)
            return jax.lax.dot_general(q2, kg[u, g], NT, preferred_element_type=f32)

        def softmax(s):
            m = jnp.max(s, axis=-1, keepdims=True)
            p = jnp.exp2(s - m)
            l = jnp.sum(p, axis=-1, keepdims=True)
            return p.astype(bf16), l

        def pv(j, p, l):
            u, g = items[j]
            o = jnp.dot(p, vg[u, g], preferred_element_type=f32)
            o = (o * pl.reciprocal(l, approx=True)).astype(bf16)
            for r in range(rep):
                qv[qslice(u, g, r)] = o[r * sq:(r + 1) * sq]

        s = qk(0)
        for j in range(n):
            s_next = qk(j + 1) if j + 1 < n else None
            p, l = softmax(s)
            pv(j, p, l)
            s = s_next

        @pl.when(i + NGRP < n2)
        def _():
            k_copy(i + NGRP, grp).start()
            v_copy(i + NGRP, grp).start()
        return carry

    jax.lax.fori_loop(0, n2, p2, 0)

    wo_copy().wait()

    def p3(j, carry):
        for t in range(MT):
            tile = j * MT + t
            r0 = pl.multiple_of(tile * 128, 128)
            acc = None
            for c in range(hkv):
                part = jax.lax.dot_general(wot_v[:, c * CB:(c + 1) * CB], q_v[c, pl.ds(r0, 128), :], NT,
                                           preferred_element_type=f32)
                acc = part if acc is None else acc + part
            out_v[pl.ds(r0, 128), :] = acc.T.astype(bf16)
            if PERTILE:
                out_copy(tile, 1, tile).start()
        if not PERTILE:
            out_copy(j * MT, MT, j).start()
        return carry

    jax.lax.fori_loop(0, n3, p3, 0)
    if PERTILE:
        for t in range(ntile):
            out_copy(t, 1, t).wait()
    else:
        for j in range(n3):
            out_copy(j * MT, MT, j).wait()


@jax.jit
def pallas_standalone__gqa_block_cached__near_ridge_kernel(x, k_cache, v_cache, wq, wo):
    B, Sq, D = x.shape
    _, Hkv, Sk, Dh = k_cache.shape
    N = wq.shape[1]
    Hq = N // Dh
    M = B * Sq
    CB = N // Hkv
    kern = functools.partial(_kernel, B=B, sq=Sq, hq=Hq, hkv=Hkv, dh=Dh)
    hbm = lambda a: pltpu.with_memory_space_constraint(a, pltpu.HBM)
    any_spec = pl.BlockSpec(memory_space=pl.ANY)
    out = pl.pallas_call(
        kern,
        in_specs=[any_spec] * 5,
        out_specs=any_spec,
        out_shape=jax.ShapeDtypeStruct((M, D), x.dtype),
        scratch_shapes=[
            pltpu.VMEM((M, D), bf16),
            pltpu.VMEM((Hkv, D, CB), bf16),
            pltpu.VMEM((D, N), bf16),
            pltpu.VMEM((Hkv, M, CB), bf16),
            pltpu.VMEM((NGRP, NB2, Hkv, Sk, Dh), bf16),
            pltpu.VMEM((NGRP, NB2, Hkv, Sk, Dh), bf16),
            pltpu.VMEM((M, D), bf16),
            pltpu.SemaphoreType.DMA((2,)),
            pltpu.SemaphoreType.DMA((Hkv,)),
            pltpu.SemaphoreType.DMA((1,)),
            pltpu.SemaphoreType.DMA((NGRP,)),
            pltpu.SemaphoreType.DMA((NGRP,)),
            pltpu.SemaphoreType.DMA((M // 128,)),
        ],
        compiler_params=pltpu.CompilerParams(
            vmem_limit_bytes=120 * 1024 * 1024,
            disable_bounds_checks=True,
            disable_semaphore_checks=True,
        ),
    )(hbm(x.reshape(M, D)), hbm(k_cache), hbm(v_cache), hbm(wq), hbm(wo.T))
    return out.reshape(B, Sq, D)
```

```python
import functools

import jax
import jax.numpy as jnp
import jax.experimental.pallas as pl
import jax.experimental.pallas.tpu as pltpu

RA = 256
RBLK = 832
NB2 = 4
NGRP = 3
MT = 4
LOG2E = 1.4426950408889634

f32 = jnp.float32
bf16 = jnp.bfloat16
NT = (((1,), (1,)), ((), ()))


def _kernel(x_hbm, k_hbm, v_hbm, wq_hbm, wot_hbm, out_hbm,
            x_v, wq_v, wot_v, q_v, k_v, v_v, out_v, pend_v,
            sem_x, sem_wq, sem_wo, sem_k, sem_v, sem_o,
            *, B, sq, hq, hkv, dh):
    M, D = x_hbm.shape
    rep = hq // hkv
    CB = rep * dh
    scale = (dh ** -0.5) * LOG2E
    n1b = (M - RA) // RBLK
    n2 = B // NB2
    ntile = M // 128
    n3 = ntile // MT
    assert RA + n1b * RBLK == M and n1b <= hkv and n2 * NB2 == B and n3 * MT == ntile

    def x0_copy():
        rows = pl.ds(0, RA)
        return pltpu.make_async_copy(x_hbm.at[rows, :], x_v.at[rows, :], sem_x.at[0])

    def x_copy(r):
        rows = pl.ds(pl.multiple_of(RA + r * RBLK, 16), RBLK)
        return pltpu.make_async_copy(x_hbm.at[rows, :], x_v.at[rows, :], sem_x.at[1 + r])

    def wq_copy(c):
        return pltpu.make_async_copy(wq_hbm.at[:, pl.ds(c * CB, CB)], wq_v.at[c], sem_wq.at[c])

    def wo_copy():
        return pltpu.make_async_copy(wot_hbm, wot_v, sem_wo.at[0])

    def k_copy(i, grp):
        return pltpu.make_async_copy(k_hbm.at[pl.ds(i * NB2, NB2)], k_v.at[grp], sem_k.at[grp])

    def v_copy(i, grp):
        return pltpu.make_async_copy(v_hbm.at[pl.ds(i * NB2, NB2)], v_v.at[grp], sem_v.at[grp])

    def out_copy(tile):
        rows = pl.ds(pl.multiple_of(tile * 128, 128), 128)
        return pltpu.make_async_copy(out_v.at[rows, :], out_hbm.at[rows, :], sem_o.at[tile])

    def qproj(r0, nrows, c):
        xb = x_v[pl.ds(r0, nrows), :]
        for t in range(rep):
            y = jnp.dot(xb, wq_v[c, :, t * dh:(t + 1) * dh], preferred_element_type=f32)
            q_v[c, pl.ds(r0, nrows), t * dh:(t + 1) * dh] = (y * scale).astype(bf16)

    x0_copy().start()
    wq_copy(0).start()
    x0_copy().wait()
    for c in range(1, hkv):
        wq_copy(c).start()

    def p1a(c, carry):
        wq_copy(c).wait()
        qproj(0, RA, c)

        @pl.when(c < n1b)
        def _():
            x_copy(c).start()
        return carry

    jax.lax.fori_loop(0, hkv, p1a, 0)

    for grp in range(NGRP):
        k_copy(grp, grp).start()
        v_copy(grp, grp).start()
        if grp == 1:
            wo_copy().start()

    def p1b(r, carry):
        x_copy(r).wait()
        r0 = pl.multiple_of(RA + r * RBLK, 16)
        for c in range(hkv):
            qproj(r0, RBLK, c)
        return carry

    jax.lax.fori_loop(0, n1b, p1b, 0)

    def p2(i, grp):
        k_copy(i, grp).wait()
        v_copy(i, grp).wait()
        kg = k_v.at[grp]
        vg = v_v.at[grp]
        r0 = pl.multiple_of(i * (NB2 * sq), 16)
        qv = q_v.at[:, pl.ds(r0, NB2 * sq), :]
        items = [(u, g) for u in range(NB2) for g in range(hkv)]
        n = len(items)

        def qslice(u, g, r):
            return (g, slice(u * sq, (u + 1) * sq), slice(r * dh, (r + 1) * dh))

        def qk(j):
            u, g = items[j]
            q2 = jnp.concatenate([qv[qslice(u, g, r)] for r in range(rep)], axis=0)
            return jax.lax.dot_general(q2, kg[u, g], NT, preferred_element_type=f32)

        def softmax(s):
            m = jnp.max(s, axis=-1, keepdims=True)
            p = jnp.exp2(s - m)
            l = jnp.sum(p, axis=-1, keepdims=True)
            return p.astype(bf16), l

        def pv(j, p, l):
            u, g = items[j]
            o = jnp.dot(p, vg[u, g], preferred_element_type=f32)
            o = (o * pl.reciprocal(l, approx=True)).astype(bf16)
            for r in range(rep):
                qv[qslice(u, g, r)] = o[r * sq:(r + 1) * sq]

        s = qk(0)
        for j in range(n):
            s_next = qk(j + 1) if j + 1 < n else None
            p, l = softmax(s)
            pv(j, p, l)
            s = s_next

        @pl.when(i + NGRP < n2)
        def _():
            k_copy(i + NGRP, grp).start()
            v_copy(i + NGRP, grp).start()
        return jnp.where(grp + 1 == NGRP, 0, grp + 1)

    jax.lax.fori_loop(0, n2, p2, jnp.int32(0))

    wo_copy().wait()

    def oproj_acc(tile):
        r0 = pl.multiple_of(tile * 128, 128)
        acc = None
        for c in range(hkv):
            part = jax.lax.dot_general(wot_v[:, c * CB:(c + 1) * CB], q_v[c, pl.ds(r0, 128), :], NT,
                                       preferred_element_type=f32)
            acc = part if acc is None else acc + part
        return acc

    def emit(tile, acc):
        out_v[pl.ds(pl.multiple_of(tile * 128, 128), 128), :] = acc.T.astype(bf16)

    pend_v[...] = jnp.zeros(pend_v.shape, f32)

    def p3(j, carry):
        prev = jnp.where(j == 0, ntile - 1, j * MT - 1)
        emit(prev, pend_v[...])

        @pl.when(j > 0)
        def _():
            out_copy(prev).start()
        for t in range(MT - 1):
            tile = j * MT + t
            emit(tile, oproj_acc(tile))
            out_copy(tile).start()
        pend_v[...] = oproj_acc(j * MT + MT - 1)
        return carry

    jax.lax.fori_loop(0, n3, p3, 0)
    emit(ntile - 1, pend_v[...])
    out_copy(ntile - 1).start()
    for t in range(ntile):
        out_copy(t).wait()


@jax.jit
def pallas_standalone__gqa_block_cached__near_ridge_kernel(x, k_cache, v_cache, wq, wo):
    B, Sq, D = x.shape
    _, Hkv, Sk, Dh = k_cache.shape
    N = wq.shape[1]
    Hq = N // Dh
    M = B * Sq
    CB = N // Hkv
    kern = functools.partial(_kernel, B=B, sq=Sq, hq=Hq, hkv=Hkv, dh=Dh)
    any_spec = pl.BlockSpec(memory_space=pl.ANY)
    out = pl.pallas_call(
        kern,
        in_specs=[any_spec] * 5,
        out_specs=any_spec,
        out_shape=jax.ShapeDtypeStruct((M, D), x.dtype),
        scratch_shapes=[
            pltpu.VMEM((M, D), bf16),
            pltpu.VMEM((Hkv, D, CB), bf16),
            pltpu.VMEM((D, N), bf16),
            pltpu.VMEM((Hkv, M, CB), bf16),
            pltpu.VMEM((NGRP, NB2, Hkv, Sk, Dh), bf16),
            pltpu.VMEM((NGRP, NB2, Hkv, Sk, Dh), bf16),
            pltpu.VMEM((M, D), bf16),
            pltpu.VMEM((D, 128), f32),
            pltpu.SemaphoreType.DMA((1 + (M - RA) // RBLK,)),
            pltpu.SemaphoreType.DMA((Hkv,)),
            pltpu.SemaphoreType.DMA((1,)),
            pltpu.SemaphoreType.DMA((NGRP,)),
            pltpu.SemaphoreType.DMA((NGRP,)),
            pltpu.SemaphoreType.DMA((M // 128,)),
        ],
        compiler_params=pltpu.CompilerParams(
            vmem_limit_bytes=126 * 1024 * 1024,
            disable_bounds_checks=True,
            disable_semaphore_checks=True,
        ),
    )(x.reshape(M, D), k_cache, v_cache, wq, wo.T)
    return out.reshape(B, Sq, D)
```

```python
import functools

import jax
import jax.numpy as jnp
import jax.experimental.pallas as pl
import jax.experimental.pallas.tpu as pltpu

RA = 256
NA1 = 4
RBLK = 832
NB2 = 4
NGRP = 4
MT = 4
LOG2E = 1.4426950408889634

f32 = jnp.float32
bf16 = jnp.bfloat16
NT = (((1,), (1,)), ((), ()))


def _kernel(x_hbm, k_hbm, v_hbm, wq_hbm, wot_hbm, out_hbm,
            x_v, wq_v, wot_v, q_v, k_v, v_v, out_v, pend_v,
            sem_x, sem_wq, sem_wo, sem_k, sem_v, sem_o,
            *, B, sq, hq, hkv, dh):
    M, D = x_hbm.shape
    rep = hq // hkv
    CB = rep * dh
    scale = (dh ** -0.5) * LOG2E
    n1b = (M - RA) // RBLK
    n2 = B // NB2
    ntile = M // 128
    n3 = ntile // MT
    assert RA + n1b * RBLK == M and n1b <= NA1 and (hkv - NA1) % 2 == 0 and n2 * NB2 == B and n3 * MT == ntile

    def x0_copy():
        rows = pl.ds(0, RA)
        return pltpu.make_async_copy(x_hbm.at[rows, :], x_v.at[rows, :], sem_x.at[0])

    def x_copy(r):
        rows = pl.ds(pl.multiple_of(RA + r * RBLK, 16), RBLK)
        return pltpu.make_async_copy(x_hbm.at[rows, :], x_v.at[rows, :], sem_x.at[1 + r])

    def wq_copy(c):
        return pltpu.make_async_copy(wq_hbm.at[:, pl.ds(c * CB, CB)], wq_v.at[c], sem_wq.at[c])

    def wo_copy():
        return pltpu.make_async_copy(wot_hbm, wot_v, sem_wo.at[0])

    def k_copy(i, grp):
        return pltpu.make_async_copy(k_hbm.at[pl.ds(i * NB2, NB2)], k_v.at[grp], sem_k.at[grp])

    def v_copy(i, grp):
        return pltpu.make_async_copy(v_hbm.at[pl.ds(i * NB2, NB2)], v_v.at[grp], sem_v.at[grp])

    def out_copy(tile):
        rows = pl.ds(pl.multiple_of(tile * 128, 128), 128)
        return pltpu.make_async_copy(out_v.at[rows, :], out_hbm.at[rows, :], sem_o.at[tile])

    def qproj(r0, nrows, c):
        xb = x_v[pl.ds(r0, nrows), :]
        for t in range(rep):
            y = jnp.dot(xb, wq_v[c, :, t * dh:(t + 1) * dh], preferred_element_type=f32)
            q_v[c, pl.ds(r0, nrows), t * dh:(t + 1) * dh] = (y * scale).astype(bf16)

    x0_copy().start()
    wq_copy(0).start()
    x0_copy().wait()
    for c in range(1, hkv):
        wq_copy(c).start()

    def p1a(c, carry):
        wq_copy(c).wait()
        qproj(0, RA, c)

        @pl.when(c < n1b)
        def _():
            x_copy(c).start()
        return carry

    jax.lax.fori_loop(0, NA1, p1a, 0)

    def p1a2(i, carry):
        c = NA1 + 2 * i
        wq_copy(c).wait()
        wq_copy(c + 1).wait()
        qproj(0, RA, c)
        qproj(0, RA, c + 1)
        return carry

    jax.lax.fori_loop(0, (hkv - NA1) // 2, p1a2, 0)

    for grp in range(NGRP):
        k_copy(grp, grp).start()
        v_copy(grp, grp).start()
        if grp == 1:
            wo_copy().start()

    def p1b(r, carry):
        x_copy(r).wait()
        r0 = pl.multiple_of(RA + r * RBLK, 16)
        for c in range(hkv):
            qproj(r0, RBLK, c)
        return carry

    jax.lax.fori_loop(0, n1b, p1b, 0)

    def p2(i, grp):
        k_copy(i, grp).wait()
        v_copy(i, grp).wait()
        kg = k_v.at[grp]
        vg = v_v.at[grp]
        r0 = pl.multiple_of(i * (NB2 * sq), 16)
        qv = q_v.at[:, pl.ds(r0, NB2 * sq), :]
        items = [(u, g) for u in range(NB2) for g in range(hkv)]
        n = len(items)

        def qslice(u, g, r):
            return (g, slice(u * sq, (u + 1) * sq), slice(r * dh, (r + 1) * dh))

        def qk(j):
            u, g = items[j]
            q2 = jnp.concatenate([qv[qslice(u, g, r)] for r in range(rep)], axis=0)
            return jax.lax.dot_general(q2, kg[u, g], NT, preferred_element_type=f32)

        def softmax(s):
            m = jnp.max(s, axis=-1, keepdims=True)
            p = jnp.exp2(s - m)
            l = jnp.sum(p, axis=-1, keepdims=True)
            return p.astype(bf16), l

        def pv(j, p, l):
            u, g = items[j]
            o = jnp.dot(p, vg[u, g], preferred_element_type=f32)
            o = (o * pl.reciprocal(l, approx=True)).astype(bf16)
            for r in range(rep):
                qv[qslice(u, g, r)] = o[r * sq:(r + 1) * sq]

        s = qk(0)
        for j in range(n):
            s_next = qk(j + 1) if j + 1 < n else None
            p, l = softmax(s)
            pv(j, p, l)
            s = s_next

        @pl.when(i + NGRP < n2)
        def _():
            k_copy(i + NGRP, grp).start()
            v_copy(i + NGRP, grp).start()
        return jnp.where(grp + 1 == NGRP, 0, grp + 1)

    jax.lax.fori_loop(0, n2, p2, jnp.int32(0))

    wo_copy().wait()

    def oproj_acc(tile):
        r0 = pl.multiple_of(tile * 128, 128)
        acc = None
        for c in range(hkv):
            part = jax.lax.dot_general(wot_v[:, c * CB:(c + 1) * CB], q_v[c, pl.ds(r0, 128), :], NT,
                                       preferred_element_type=f32)
            acc = part if acc is None else acc + part
        return acc

    def emit(tile, acc):
        out_v[pl.ds(pl.multiple_of(tile * 128, 128), 128), :] = acc.T.astype(bf16)

    pend_v[...] = jnp.zeros(pend_v.shape, f32)

    def p3(j, carry):
        prev = jnp.where(j == 0, ntile - 1, j * MT - 1)
        emit(prev, pend_v[...])

        @pl.when(j > 0)
        def _():
            out_copy(prev).start()
        for t in range(MT - 1):
            tile = j * MT + t
            emit(tile, oproj_acc(tile))
            out_copy(tile).start()
        pend_v[...] = oproj_acc(j * MT + MT - 1)
        return carry

    jax.lax.fori_loop(0, n3, p3, 0)
    emit(ntile - 1, pend_v[...])
    out_copy(ntile - 1).start()
    for t in range(ntile):
        out_copy(t).wait()


@jax.jit
def pallas_standalone__gqa_block_cached__near_ridge_kernel(x, k_cache, v_cache, wq, wo):
    B, Sq, D = x.shape
    _, Hkv, Sk, Dh = k_cache.shape
    N = wq.shape[1]
    Hq = N // Dh
    M = B * Sq
    CB = N // Hkv
    kern = functools.partial(_kernel, B=B, sq=Sq, hq=Hq, hkv=Hkv, dh=Dh)
    any_spec = pl.BlockSpec(memory_space=pl.ANY)
    out = pl.pallas_call(
        kern,
        in_specs=[any_spec] * 5,
        out_specs=any_spec,
        out_shape=jax.ShapeDtypeStruct((M, D), x.dtype),
        scratch_shapes=[
            pltpu.VMEM((M, D), bf16),
            pltpu.VMEM((Hkv, D, CB), bf16),
            pltpu.VMEM((D, N), bf16),
            pltpu.VMEM((Hkv, M, CB), bf16),
            pltpu.VMEM((NGRP, NB2, Hkv, Sk, Dh), bf16),
            pltpu.VMEM((NGRP, NB2, Hkv, Sk, Dh), bf16),
            pltpu.VMEM((M, D), bf16),
            pltpu.VMEM((D, 128), f32),
            pltpu.SemaphoreType.DMA((1 + (M - RA) // RBLK,)),
            pltpu.SemaphoreType.DMA((Hkv,)),
            pltpu.SemaphoreType.DMA((1,)),
            pltpu.SemaphoreType.DMA((NGRP,)),
            pltpu.SemaphoreType.DMA((NGRP,)),
            pltpu.SemaphoreType.DMA((M // 128,)),
        ],
        compiler_params=pltpu.CompilerParams(
            vmem_limit_bytes=126 * 1024 * 1024,
            disable_bounds_checks=True,
            disable_semaphore_checks=True,
        ),
    )(x.reshape(M, D), k_cache, v_cache, wq, wo.T)
    return out.reshape(B, Sq, D)
```

```python
import functools

import jax
import jax.numpy as jnp
import jax.experimental.pallas as pl
import jax.experimental.pallas.tpu as pltpu

RA = 320
CM = 1
NA1 = 3
RBLK = 816
NB2 = 4
NGRP = 4
MT = 4
LOG2E = 1.4426950408889634

f32 = jnp.float32
bf16 = jnp.bfloat16
NT = (((1,), (1,)), ((), ()))


def _kernel(x_hbm, k_hbm, v_hbm, wq_hbm, wot_hbm, out_hbm,
            x_v, wq_v, wot_v, q_v, k_v, v_v, out_v, pend_v,
            sem_x, sem_wq, sem_wo, sem_k, sem_v, sem_o,
            *, B, sq, hq, hkv, dh):
    M, D = x_hbm.shape
    rep = hq // hkv
    CB = rep * dh
    scale = (dh ** -0.5) * LOG2E
    n1b = (M - RA) // RBLK
    n2 = B // NB2
    ntile = M // 128
    n3 = ntile // MT
    assert RA + n1b * RBLK == M and n1b <= hkv and (hkv - CM - NA1) % 2 == 0 and n2 * NB2 == B and n3 * MT == ntile

    def x0_copy():
        rows = pl.ds(0, RA)
        return pltpu.make_async_copy(x_hbm.at[rows, :], x_v.at[rows, :], sem_x.at[0])

    def x_copy(r):
        rows = pl.ds(pl.multiple_of(RA + r * RBLK, 16), RBLK)
        return pltpu.make_async_copy(x_hbm.at[rows, :], x_v.at[rows, :], sem_x.at[1 + r])

    def wq_copy(c):
        return pltpu.make_async_copy(wq_hbm.at[:, pl.ds(c * CB, CB)], wq_v.at[c], sem_wq.at[c])

    def wo_copy():
        return pltpu.make_async_copy(wot_hbm, wot_v, sem_wo.at[0])

    def k_copy(i, grp):
        return pltpu.make_async_copy(k_hbm.at[pl.ds(i * NB2, NB2)], k_v.at[grp], sem_k.at[grp])

    def v_copy(i, grp):
        return pltpu.make_async_copy(v_hbm.at[pl.ds(i * NB2, NB2)], v_v.at[grp], sem_v.at[grp])

    def out_copy(tile):
        rows = pl.ds(pl.multiple_of(tile * 128, 128), 128)
        return pltpu.make_async_copy(out_v.at[rows, :], out_hbm.at[rows, :], sem_o.at[tile])

    def qproj(r0, nrows, c):
        xb = x_v[pl.ds(r0, nrows), :]
        for t in range(rep):
            y = jnp.dot(xb, wq_v[c, :, t * dh:(t + 1) * dh], preferred_element_type=f32)
            q_v[c, pl.ds(r0, nrows), t * dh:(t + 1) * dh] = (y * scale).astype(bf16)

    x0_copy().start()
    wq_copy(0).start()
    x0_copy().wait()
    for c in range(1, hkv):
        wq_copy(c).start()

    def p1a(c, carry):
        wq_copy(c).wait()
        qproj(0, RA, c)

        @pl.when(c < n1b)
        def _():
            x_copy(c).start()
        return carry

    jax.lax.fori_loop(0, NA1, p1a, 0)
    for r in range(NA1, n1b):
        x_copy(r).start()

    def p1a2(i, carry):
        c = NA1 + 2 * i
        wq_copy(c).wait()
        wq_copy(c + 1).wait()
        qproj(0, RA, c)
        qproj(0, RA, c + 1)
        return carry

    jax.lax.fori_loop(0, (hkv - CM - NA1) // 2, p1a2, 0)

    for grp in range(NGRP):
        k_copy(grp, grp).start()
        v_copy(grp, grp).start()
        if grp == 1:
            wo_copy().start()

    def p1b(r, carry):
        x_copy(r).wait()
        r0 = pl.multiple_of(RA + r * RBLK, 16)
        for c in range(hkv - CM):
            qproj(r0, RBLK, c)
        return carry

    jax.lax.fori_loop(0, n1b, p1b, 0)
    for c in range(hkv - CM, hkv):
        wq_copy(c).wait()

    def p2(i, grp):
        k_copy(i, grp).wait()
        v_copy(i, grp).wait()
        kg = k_v.at[grp]
        vg = v_v.at[grp]
        r0 = pl.multiple_of(i * (NB2 * sq), 16)
        qv = q_v.at[:, pl.ds(r0, NB2 * sq), :]
        for c in range(hkv - CM, hkv):
            qproj(r0, NB2 * sq, c)
        items = [(u, g) for u in range(NB2) for g in range(hkv)]
        n = len(items)

        def qslice(u, g, r):
            return (g, slice(u * sq, (u + 1) * sq), slice(r * dh, (r + 1) * dh))

        def qk(j):
            u, g = items[j]
            q2 = jnp.concatenate([qv[qslice(u, g, r)] for r in range(rep)], axis=0)
            return jax.lax.dot_general(q2, kg[u, g], NT, preferred_element_type=f32)

        def softmax(s):
            m = jnp.max(s, axis=-1, keepdims=True)
            p = jnp.exp2(s - m)
            l = jnp.sum(p, axis=-1, keepdims=True)
            return p.astype(bf16), l

        def pv(j, p, l):
            u, g = items[j]
            o = jnp.dot(p, vg[u, g], preferred_element_type=f32)
            o = (o * pl.reciprocal(l, approx=True)).astype(bf16)
            for r in range(rep):
                qv[qslice(u, g, r)] = o[r * sq:(r + 1) * sq]

        s = qk(0)
        for j in range(n):
            s_next = qk(j + 1) if j + 1 < n else None
            p, l = softmax(s)
            pv(j, p, l)
            s = s_next

        @pl.when(i + NGRP < n2)
        def _():
            k_copy(i + NGRP, grp).start()
            v_copy(i + NGRP, grp).start()
        return jnp.where(grp + 1 == NGRP, 0, grp + 1)

    jax.lax.fori_loop(0, n2, p2, jnp.int32(0))

    wo_copy().wait()

    def oproj_acc(tile):
        r0 = pl.multiple_of(tile * 128, 128)
        acc = None
        for c in range(hkv):
            part = jax.lax.dot_general(wot_v[:, c * CB:(c + 1) * CB], q_v[c, pl.ds(r0, 128), :], NT,
                                       preferred_element_type=f32)
            acc = part if acc is None else acc + part
        return acc

    def emit(tile, acc):
        out_v[pl.ds(pl.multiple_of(tile * 128, 128), 128), :] = acc.T.astype(bf16)

    pend_v[...] = jnp.zeros(pend_v.shape, f32)

    def p3(j, carry):
        prev = jnp.where(j == 0, ntile - 1, j * MT - 1)
        emit(prev, pend_v[...])

        @pl.when(j > 0)
        def _():
            out_copy(prev).start()
        for t in range(MT - 1):
            tile = j * MT + t
            emit(tile, oproj_acc(tile))
            out_copy(tile).start()
        pend_v[...] = oproj_acc(j * MT + MT - 1)
        return carry

    jax.lax.fori_loop(0, n3, p3, 0)
    emit(ntile - 1, pend_v[...])
    out_copy(ntile - 1).start()
    for t in range(ntile):
        out_copy(t).wait()


@jax.jit
def pallas_standalone__gqa_block_cached__near_ridge_kernel(x, k_cache, v_cache, wq, wo):
    B, Sq, D = x.shape
    _, Hkv, Sk, Dh = k_cache.shape
    N = wq.shape[1]
    Hq = N // Dh
    M = B * Sq
    CB = N // Hkv
    kern = functools.partial(_kernel, B=B, sq=Sq, hq=Hq, hkv=Hkv, dh=Dh)
    any_spec = pl.BlockSpec(memory_space=pl.ANY)
    out = pl.pallas_call(
        kern,
        in_specs=[any_spec] * 5,
        out_specs=any_spec,
        out_shape=jax.ShapeDtypeStruct((M, D), x.dtype),
        scratch_shapes=[
            pltpu.VMEM((M, D), bf16),
            pltpu.VMEM((Hkv, D, CB), bf16),
            pltpu.VMEM((D, N), bf16),
            pltpu.VMEM((Hkv, M, CB), bf16),
            pltpu.VMEM((NGRP, NB2, Hkv, Sk, Dh), bf16),
            pltpu.VMEM((NGRP, NB2, Hkv, Sk, Dh), bf16),
            pltpu.VMEM((M, D), bf16),
            pltpu.VMEM((D, 128), f32),
            pltpu.SemaphoreType.DMA((1 + (M - RA) // RBLK,)),
            pltpu.SemaphoreType.DMA((Hkv,)),
            pltpu.SemaphoreType.DMA((1,)),
            pltpu.SemaphoreType.DMA((NGRP,)),
            pltpu.SemaphoreType.DMA((NGRP,)),
            pltpu.SemaphoreType.DMA((M // 128,)),
        ],
        compiler_params=pltpu.CompilerParams(
            vmem_limit_bytes=126 * 1024 * 1024,
            disable_bounds_checks=True,
            disable_semaphore_checks=True,
        ),
    )(x.reshape(M, D), k_cache, v_cache, wq, wo.T)
    return out.reshape(B, Sq, D)
```
